```python
import os as _os
_os.environ.setdefault("JAX_PLATFORMS", "cpu")
import jax
import jax.numpy as jnp

def _softmax(x, axis=-1):
    return jax.nn.softmax(x, axis=axis)
def _gelu(x):
    return jax.nn.gelu(x, approximate=True)
def _silu(x):
    return jax.nn.silu(x)
def _sigmoid(x):
    return jax.nn.sigmoid(x)
def _layernorm(x, axis=-1, eps=1e-5):
    m = jnp.mean(x, axis=axis, keepdims=True)
    v = jnp.var(x, axis=axis, keepdims=True)
    return (x - m) / jnp.sqrt(v + eps)
def _scatter_add(tgt, idx, src, axis=0):
    return tgt.at[idx].add(src)
def _segment_sum(src, seg, n):
    return jax.ops.segment_sum(src, seg, n)
class _Rng:
    def __init__(self, key):
        self._k = key
    def _next(self):
        self._k, sub = jax.random.split(self._k)
        return sub
    def normal(self, shape):
        return jax.random.normal(self._next(), shape, dtype=jnp.bfloat16)
    def randint(self, lo, hi, shape):
        return jax.random.randint(self._next(), shape, lo, hi, dtype=jnp.int32)
    def uniform(self, shape, lo=0.0, hi=1.0):
        return jax.random.uniform(self._next(), shape, jnp.bfloat16, lo, hi)
    def permutation(self, n):
        return jax.random.permutation(self._next(), n)


kernel_name = 'interleave_layers__sliding_block__dense_activation_gelu__prompt'

def setup_inputs():
    _rng = _Rng(jax.random.key(int.from_bytes(__import__("os").urandom(4), "little")))
    _w = (lambda a: (lambda t: t.astype(jnp.bfloat16) if jnp.issubdtype(t.dtype, jnp.floating) else t)(jnp.asarray(a)))
    def _A_setup():
        B, S, D = 1, 2048, 640
        return {
            "x": _w((lambda *s: _rng.normal(s) * 0.05)(B, S, D)),
            "wqkv": _w((lambda *s: _rng.normal(s) * 0.05)(D, 3 * D)),
            "wo": _w((lambda *s: _rng.normal(s) * 0.05)(D, D)),
        }
    _A_in = _A_setup()

    def _B_setup():
        B, S, D, F = 1, 2048, 640, 1728
        return {
            "x": _w((lambda *s: _rng.normal(s) * 0.05)(B, S, D)),
            "w1": _w((lambda *s: _rng.normal(s) * 0.8)(D, F) * (D ** -0.5)),
            "b1": _w((lambda *s: _rng.normal(s) * 0.8)(F) * 0.01),
            "w2": _w((lambda *s: _rng.normal(s) * 0.8)(F, D) * (F ** -0.5)),
            "b2": _w((lambda *s: _rng.normal(s) * 0.8)(D) * 0.01),
        }
    _B_in = _B_setup()

    return {
        "A_x": _A_in["x"],
        "A_wqkv": _A_in["wqkv"],
        "A_wo": _A_in["wo"],
        "B_x": _B_in["x"],
        "B_w1": _B_in["w1"],
        "B_b1": _B_in["b1"],
        "B_w2": _B_in["w2"],
        "B_b2": _B_in["b2"],
    }

def reference(A_x, A_wqkv, A_wo, B_x, B_w1, B_b1, B_w2, B_b2):
    def _A_ref(x, wqkv, wo):
        B, S, D = x.shape
        H = 32; Dh = D // H; W = 256
        qkv = (lambda x, *d: x.transpose(*d))((x @ wqkv).reshape(B, S, 3, H, Dh), 2, 0, 3, 1, 4)
        q, k, v = qkv[0], qkv[1], qkv[2]
        scores = jnp.einsum("bhqd,bhkd->bhqk", q, k) * (Dh ** -0.5)
        idx = jnp.arange(S)
        mask = (idx[:, None] - idx[None, :] >= 0) & (idx[:, None] - idx[None, :] < W)
        scores = jnp.where(mask[None, None], scores, -1e9)
        p = _softmax(scores, axis=-1)
        o = jnp.einsum("bhqk,bhkd->bhqd", p, v)
        return (lambda x, *d: x.transpose(*d))(o, 0, 2, 1, 3).reshape(B, S, D) @ wo

    def _B_ref(x, w1, b1, w2, b2):
        h = jnp.einsum("bsd,df->bsf", x, w1) + b1
        h = _gelu(h)
        return jnp.einsum("bsf,fd->bsd", h, w2) + b2

    x = A_x
    x = x + _A_ref(_layernorm(x, axis=-1), A_wqkv, A_wo)
    x = x + _B_ref(_layernorm(x, axis=-1), B_w1, B_b1, B_w2, B_b2)
    x = x + _A_ref(_layernorm(x, axis=-1), A_wqkv, A_wo)
    x = x + _B_ref(_layernorm(x, axis=-1), B_w1, B_b1, B_w2, B_b2)
    return x
```

```python
import jax
import jax.numpy as jnp
from jax import lax
import jax.experimental.pallas as pl
import jax.experimental.pallas.tpu as pltpu

S, D, F, H, DH, W = 2048, 640, 1728, 32, 20, 256
RC = 512
NG = 8
WIN = (0, 64, 128, 192, 320, 384, 448, 512)
BF, F32 = jnp.bfloat16, jnp.float32
NT = (((1,), (1,)), ((), ()))
QSCALE = (DH ** -0.5) * 1.4426950408889634


def _ln(x):
    m = jnp.mean(x, axis=-1, keepdims=True)
    c = x - m
    v = jnp.mean(c * c, axis=-1, keepdims=True)
    return (c * lax.rsqrt(v + 1e-5)).astype(BF)


def _kernel(x_hbm, wqkv_hbm, wo_hbm, w1_hbm, b1_ref, w2_hbm, b2_ref, out_hbm,
            x_ref, wqkv_ref, wo_ref, w1_ref, w2_ref, sems, osems,
            xs, qw, kw, vT, ow, wvT, s0, s1, p0, p1, l0, l1):
    cps = [pltpu.make_async_copy(src, dst, sems.at[i]) for i, (src, dst) in enumerate(
        [(wqkv_hbm, wqkv_ref), (x_hbm, x_ref), (wo_hbm, wo_ref), (w1_hbm, w1_ref),
         (w2_hbm, w2_ref)])]
    for cp in cps:
        cp.start()
    for g in range(NG):
        pad = lax.broadcasted_iota(jnp.int32, (W, 128), 1) == ((g % 4) * 16 + 80) % 128
        kw[g, :W, :] = jnp.where(pad, -1e30, 0.0).astype(BF)
    p0[...] = jnp.zeros(p0.shape, BF)
    p1[...] = jnp.zeros(p1.shape, BF)
    vT[:, :W] = jnp.zeros((D, W), BF)
    cps[0].wait()
    wvT[...] = wqkv_ref[:, 2 * D:].T
    cps[1].wait()

    @pl.loop(0, S // RC)
    def _(i):
        r = pl.ds(pl.multiple_of(i * RC, RC), RC)
        xs[r, :] = x_ref[r, :].astype(F32)

    def qkv(i):
        r0 = pl.multiple_of(i * RC, RC)
        r = pl.ds(r0, RC)
        xn = _ln(xs[r, :])
        q = jnp.dot(xn, wqkv_ref[:, :D], preferred_element_type=F32) * QSCALE
        k = jnp.dot(xn, wqkv_ref[:, D:2 * D], preferred_element_type=F32)
        spare = lax.broadcasted_iota(jnp.int32, (RC, 128), 1)
        for g in range(NG):
            qw[g, r, :] = q[:, WIN[g]:WIN[g] + 128].astype(BF)
            kw[g, pl.ds(r0 + W, RC), :] = jnp.where(
                spare == ((g % 4) * 16 + 80) % 128, 0.0, k[:, WIN[g]:WIN[g] + 128]).astype(BF)
        v = lax.dot_general(wvT[...], xn, NT, preferred_element_type=F32)
        vT[:, pl.ds(pl.multiple_of(r0 + W, 128), RC)] = v.astype(BF)

    lane = lax.broadcasted_iota(jnp.int32, (32, 128), 1)
    row = lax.broadcasted_iota(jnp.int32, (32, 128), 0)

    def split(n):
        n = jnp.asarray(n, jnp.int32)
        return n >> 4, pl.multiple_of((n & 15) * 128, 128)

    def scores(n, s_ref):
        g, t0 = split(n)
        off = (g & 3) * 16
        ln = lane[:16]
        one = jnp.where(ln == ((off + 80) & 127), 0x3F803F80, 0)
        hm = [(ln >= off + DH * h) & (ln < off + DH * (h + 1)) for h in range(4)]
        for j in range(4):
            q0 = pl.multiple_of(t0 + 32 * j, 32)
            q32 = pltpu.bitcast(qw[g, pl.ds(q0, 32), :], jnp.int32)
            qbd = pltpu.bitcast(
                jnp.concatenate([jnp.where(hm[h], q32, one) for h in range(4)], axis=0), BF)
            s_ref[j] = lax.dot_general(kw[g, pl.ds(q0, 288), :], qbd, NT,
                                       preferred_element_type=F32)

    def softmax(s_ref, p_ref, l_ref):
        c = lane & 31
        for j in range(4):
            parts = [s_ref[j, a:a + 32, :] for a in range(0, 288, 32)]
            parts[0] = jnp.where(row > c, parts[0], -1e30)
            parts[-1] = jnp.where(row <= c, parts[-1], -1e30)
            m = parts[0]
            for p_ in parts[1:]:
                m = jnp.maximum(m, p_)
            m = jnp.max(m, axis=0, keepdims=True)
            l = None
            for a, p_ in enumerate(parts):
                e = jnp.exp2(p_ - m)
                l = e if l is None else l + e
                p_ref[j, 32 * (j + a):32 * (j + a + 1), :] = e.astype(BF)
            l_ref[j] = jnp.broadcast_to(1.0 / jnp.sum(l, axis=0, keepdims=True), (8, 128))

    def values(n, p_ref, l_ref):
        g, t0 = split(n)
        vt = vT[pl.ds(pl.multiple_of(g * 80, 16), 80), pl.ds(t0, 384)]
        for j in range(4):
            oT = jnp.dot(vt, p_ref[j], preferred_element_type=F32) * l_ref[j, 0:1, :]
            o = jnp.concatenate([oT, jnp.zeros((48, 128), F32)], axis=0).T
            o = jnp.where(lane < DH, o[0:32], jnp.where(lane < 2 * DH, o[32:64],
                          jnp.where(lane < 3 * DH, o[64:96], o[96:128])))
            ow[g, pl.ds(pl.multiple_of(t0 + 32 * j, 32), 32), :] = o.astype(BF)

    def attn():
        nt = NG * S // 128
        scores(0, s0)
        scores(1, s1)
        softmax(s0, p0, l0)

        @pl.loop(0, nt // 2 - 1, unroll=21)
        def _(i):
            n = 2 * i
            scores(n + 2, s0)
            softmax(s1, p1, l1)
            values(n, p0, l0)
            scores(n + 3, s1)
            softmax(s0, p0, l0)
            values(n + 1, p1, l1)

        softmax(s1, p1, l1)
        values(nt - 2, p0, l0)
        values(nt - 1, p1, l1)

    def proj_ffn(i):
        r = pl.ds(pl.multiple_of(i * RC, RC), RC)
        o = jnp.concatenate([ow[g, r, :][:, :80] for g in range(NG)], axis=1)
        x = xs[r, :] + jnp.dot(o, wo_ref[...], preferred_element_type=F32)
        h = lax.dot_general(_ln(x), w1_ref[...], NT, preferred_element_type=F32) + b1_ref[...].astype(F32).reshape(1, F)
        h = jax.nn.gelu(h, approximate=True).astype(BF)
        xs[r, :] = x + jnp.dot(h, w2_ref[...], preferred_element_type=F32) + b2_ref[...].astype(F32).reshape(1, D)

    @pl.loop(0, 2)
    def _(layer):
        pl.loop(0, S // RC)(qkv)
        attn()

        @pl.when(layer == 0)
        def _():
            for cp in cps[2:]:
                cp.wait()

        pl.loop(0, S // RC)(proj_ffn)

    ocs = []
    for i in range(S // RC):
        r = pl.ds(i * RC, RC)
        x_ref[r, :] = xs[r, :].astype(BF)
        ocs.append(pltpu.make_async_copy(x_ref.at[r], out_hbm.at[r], osems.at[i]))
        ocs[-1].start()
    for cp in ocs:
        cp.wait()


@jax.jit
def pallas_interleave_layers__sliding_block__dense_activation_gelu__prompt_kernel(
    A_x, A_wqkv, A_wo, B_x, B_w1, B_b1, B_w2, B_b2,
):
    del B_x
    hbm = pl.BlockSpec(memory_space=pl.ANY)
    out = pl.pallas_call(
        _kernel,
        out_shape=jax.ShapeDtypeStruct((S, D), A_x.dtype),
        in_specs=[hbm, hbm, hbm, hbm, pl.BlockSpec(), hbm, pl.BlockSpec()],
        out_specs=hbm,
        scratch_shapes=[
            pltpu.VMEM((S, D), BF),
            pltpu.VMEM((D, 3 * D), BF),
            pltpu.VMEM((D, D), BF),
            pltpu.VMEM((F, D), BF),
            pltpu.VMEM((F, D), BF),
            pltpu.SemaphoreType.DMA((5,)),
            pltpu.SemaphoreType.DMA((S // RC,)),
            pltpu.VMEM((S, D), F32),
            pltpu.VMEM((NG, S, 128), BF),
            pltpu.VMEM((NG, S + W, 128), BF),
            pltpu.VMEM((D, S + W), BF),
            pltpu.VMEM((NG, S, 128), BF),
            pltpu.VMEM((D, D), BF),
            pltpu.VMEM((4, 288, 128), F32),
            pltpu.VMEM((4, 288, 128), F32),
            pltpu.VMEM((4, 384, 128), BF),
            pltpu.VMEM((4, 384, 128), BF),
            pltpu.VMEM((4, 8, 128), F32),
            pltpu.VMEM((4, 8, 128), F32),
        ],
        compiler_params=pltpu.CompilerParams(vmem_limit_bytes=100 * 1024 * 1024),
    )(A_x.reshape(S, D), A_wqkv, A_wo, B_w1.T, B_b1, B_w2, B_b2)
    return out.reshape(1, S, D)
```
